```python
import os as _os
_os.environ.setdefault("JAX_PLATFORMS", "cpu")
import jax
import jax.numpy as jnp

def _softmax(x, axis=-1):
    return jax.nn.softmax(x, axis=axis)
def _gelu(x):
    return jax.nn.gelu(x, approximate=True)
def _silu(x):
    return jax.nn.silu(x)
def _sigmoid(x):
    return jax.nn.sigmoid(x)
def _layernorm(x, axis=-1, eps=1e-5):
    m = jnp.mean(x, axis=axis, keepdims=True)
    v = jnp.var(x, axis=axis, keepdims=True)
    return (x - m) / jnp.sqrt(v + eps)
def _scatter_add(tgt, idx, src, axis=0):
    return tgt.at[idx].add(src)
def _segment_sum(src, seg, n):
    return jax.ops.segment_sum(src, seg, n)
class _Rng:
    def __init__(self, key):
        self._k = key
    def _next(self):
        self._k, sub = jax.random.split(self._k)
        return sub
    def normal(self, shape):
        return jax.random.normal(self._next(), shape, dtype=jnp.bfloat16)
    def randint(self, lo, hi, shape):
        return jax.random.randint(self._next(), shape, lo, hi, dtype=jnp.int32)
    def uniform(self, shape, lo=0.0, hi=1.0):
        return jax.random.uniform(self._next(), shape, jnp.bfloat16, lo, hi)
    def permutation(self, n):
        return jax.random.permutation(self._next(), n)


kernel_name = 'interleave_layers__grouped_kv_mqa__dense_activation_relu__prompt'

def setup_inputs():
    _rng = _Rng(jax.random.key(int.from_bytes(__import__("os").urandom(4), "little")))
    _w = (lambda a: (lambda t: t.astype(jnp.bfloat16) if jnp.issubdtype(t.dtype, jnp.floating) else t)(jnp.asarray(a)))
    def _A_setup():
        B, S, D, H = 1, 2048, 448, 16
        Dh = D // H
        return {
            "x": _w((lambda *s: _rng.normal(s) * 0.05)(B, S, D)),
            "wq": _w((lambda *s: _rng.normal(s) * 0.05)(D, H * Dh)),
            "wk": _w((lambda *s: _rng.normal(s) * 0.05)(D, Dh)),
            "wv": _w((lambda *s: _rng.normal(s) * 0.05)(D, Dh)),
            "wo": _w((lambda *s: _rng.normal(s) * 0.05)(H * Dh, D)),
        }
    _A_in = _A_setup()

    def _B_setup():
        B, S, D, Dff = 1, 2048, 448, 1792
        return {
            "x": _w((lambda *s: _rng.normal(s) * 0.05)(B, S, D)),
            "w1": _w((lambda *s: _rng.normal(s) * 0.05)(D, Dff)),
            "w2": _w((lambda *s: _rng.normal(s) * 0.05)(Dff, D)),
        }
    _B_in = _B_setup()

    return {
        "A_x": _A_in["x"],
        "A_wq": _A_in["wq"],
        "A_wk": _A_in["wk"],
        "A_wv": _A_in["wv"],
        "A_wo": _A_in["wo"],
        "B_x": _B_in["x"],
        "B_w1": _B_in["w1"],
        "B_w2": _B_in["w2"],
    }

def reference(A_x, A_wq, A_wk, A_wv, A_wo, B_x, B_w1, B_w2):
    def _A_ref(x, wq, wk, wv, wo):
        B, S, D = x.shape
        H = 16
        Dh = D // H
        q = (lambda x, *d: x.transpose(*d))((x @ wq).reshape(B, S, H, Dh), 0, 2, 1, 3)
        k = x @ wk
        v = x @ wv
        scores = jnp.einsum("bhqd,bkd->bhqk", q, k) * (Dh ** -0.5)
        p = _softmax(scores, axis=-1)
        o = jnp.einsum("bhqk,bkd->bhqd", p, v)
        return (lambda x, *d: x.transpose(*d))(o, 0, 2, 1, 3).reshape(B, S, H * Dh) @ wo

    def _B_ref(x, w1, w2):
        h = jnp.einsum("bsd,df->bsf", x, w1)
        zero = jnp.zeros_like(h)
        h = jnp.maximum(h, zero)
        return jnp.einsum("bsf,fd->bsd", h, w2)

    x = A_x
    x = x + _A_ref(_layernorm(x, axis=-1), A_wq, A_wk, A_wv, A_wo)
    x = x + _B_ref(_layernorm(x, axis=-1), B_w1, B_w2)
    x = x + _A_ref(_layernorm(x, axis=-1), A_wq, A_wk, A_wv, A_wo)
    x = x + _B_ref(_layernorm(x, axis=-1), B_w1, B_w2)
    return x
```

```python
import jax
import jax.numpy as jnp
from jax import lax
import jax.experimental.pallas as pl
import jax.experimental.pallas.tpu as pltpu

f32 = jnp.float32
bf16 = jnp.bfloat16
u32 = jnp.uint32

S = 2048
D = 448
H = 16
DH = 28
DFF = 1792
TB = 512
NT = S // TB
CH = 256
NCH = S // CH
EP = 16
HU = 2
UPT = H // HU
NU = UPT * NT
QSCALE = float(DH ** -0.5 * 1.4426950408889634)
EPS = 1e-5


def _pack(x_bf16):
    return pltpu.bitcast(x_bf16, u32)


def _unpack(x_u32):
    return pltpu.bitcast(x_u32, bf16)


def _ln_t(x):
    m = jnp.mean(x, axis=0, keepdims=True)
    d = x - m
    v = jnp.mean(d * d, axis=0, keepdims=True)
    return d * lax.rsqrt(v + EPS)


def _dot(a, b):
    return jnp.dot(a, b, preferred_element_type=f32)


def _kernel(x_hbm, wq_hbm, wk_hbm, wv_hbm, wo_hbm, w1_hbm, w2_hbm, o_hbm,
            xin_ref, wq_in, wk_in, wv_in, wo_in, w1_in, w2t_ref, obuf_ref, sems,
            xt_ref, wqt_ref, wkv_ref, wot_ref, w1t_ref, wtmp_ref,
            qt_ref, kp_ref, vt_ref, ot_ref, *bufs):
    sb = (bufs[0:HU], bufs[HU:2 * HU])
    pb = (bufs[2 * HU:3 * HU], bufs[3 * HU:4 * HU])
    mb = (bufs[4 * HU:5 * HU], bufs[5 * HU:6 * HU])
    accb = bufs[6 * HU:7 * HU]

    def x_copy(t):
        return pltpu.make_async_copy(x_hbm.at[:, t * TB:(t + 1) * TB], xin_ref.at[t], sems.at[t])

    def o_copy(t):
        c0 = pl.multiple_of(t * TB, TB)
        return pltpu.make_async_copy(obuf_ref.at[t], o_hbm.at[:, pl.ds(c0, TB)], sems.at[10 + t])

    cp_wq = pltpu.make_async_copy(wq_hbm, wq_in, sems.at[4])
    cp_wk = pltpu.make_async_copy(wk_hbm, wk_in, sems.at[5])
    cp_wv = pltpu.make_async_copy(wv_hbm, wv_in, sems.at[6])
    cp_wo = pltpu.make_async_copy(wo_hbm, wo_in, sems.at[7])
    cp_w1 = pltpu.make_async_copy(w1_hbm, w1_in, sems.at[8])
    cp_w2 = pltpu.make_async_copy(w2_hbm, w2t_ref, sems.at[9])
    cp_wk.start()
    cp_wv.start()
    x_copy(0).start()
    cp_wq.start()
    for t in range(1, NT):
        x_copy(t).start()
    cp_wo.start()
    cp_w1.start()
    cp_w2.start()

    qt_ref[...] = jnp.zeros(qt_ref.shape, u32)
    wtmp_ref[...] = jnp.zeros(wtmp_ref.shape, f32)
    cp_wk.wait()
    cp_wv.wait()
    wtmp_ref[0:DH, :] = wk_in[...].astype(f32)
    wtmp_ref[32:32 + DH, :] = wv_in[...].astype(f32)
    wkv_ref[...] = wtmp_ref[0:64, :].astype(bf16)
    cp_wq.wait()
    wqt_ref[...] = wq_in[...].T

    def qkv(t, x, lbuf):
        xn = _ln_t(x).astype(bf16)
        rkv = _dot(wkv_ref[...], xn)
        kt = jnp.concatenate([rkv[0:32, :], jnp.zeros((96, TB), f32)], axis=0)
        k = kt.T
        row0 = pl.multiple_of(t * (TB // 2), TB // 2)
        for c in range(4):
            kc = k if c == 0 else pltpu.roll(k, c * DH, 1)
            kp_ref[lbuf, c, pl.ds(row0, TB // 2), :] = _pack(kc.astype(bf16))
        v = rkv[32:64, :]
        rows = lax.broadcasted_iota(jnp.int32, (32, TB), 0)
        v = jnp.where(rows == DH, 1.0, v)
        vt_ref[lbuf, t] = _pack(v.astype(bf16))
        rq = _dot(wqt_ref[...], xn)
        for g in range(4):
            qg = (rq[g * 112:(g + 1) * 112, :] * QSCALE).astype(bf16)
            qt_ref[t, g, 0:56, :] = _pack(qg)

    for t in range(NT):
        x_copy(t).wait()
        x = xin_ref[t].astype(f32)
        xt_ref[t] = x
        qkv(t, x, 0)
        if t == 0:
            cp_wo.wait()
            wtmp_ref[0:64, :] = jnp.zeros((64, D), f32)
            wo32 = wo_in[...].astype(f32)
            for h in range(H):
                wtmp_ref[h * 32:h * 32 + DH, :] = wo32[h * DH:(h + 1) * DH, :]
            wot_ref[...] = wtmp_ref[...].astype(bf16).T
        if t == 1:
            cp_w1.wait()
            w1t_ref[0:896, :] = w1_in[:, 0:896].T
        if t == 2:
            w1t_ref[896:DFF, :] = w1_in[:, 896:DFF].T
    cp_w2.wait()

    def head_of(u, k):
        t = lax.shift_right_logical(u, UPT.bit_length() - 1)
        h = (u & (UPT - 1)) * HU + k
        return t, h

    def stage1(l, u, slot, k, j):
        t, h = head_of(u, k)
        g = lax.shift_right_logical(h, 2)
        c = h & 3
        qw = _unpack(qt_ref[t, g])
        kc = _unpack(kp_ref[l, c, j * (CH // 2):(j + 1) * (CH // 2), :])
        s = _dot(kc, qw)
        sb[slot][k][j * CH:(j + 1) * CH, :] = s
        return jnp.max(s.reshape(CH // 8, 8, TB), axis=0)

    def stage2(slot, k, m, j):
        for r in range(j * CH, (j + 1) * CH, EP):
            p = jnp.exp2(sb[slot][k][r:r + EP, :] - m).astype(bf16)
            pb[slot][k][r // 2:(r + EP) // 2, :] = _pack(p)

    def stage3(l, slot, k, j):
        p = _unpack(pb[slot][k][j * (CH // 2):(j + 1) * (CH // 2), :])
        tt = (j * CH) // TB
        c0 = (j * CH) % TB
        v = _unpack(vt_ref[l, tt, :, c0:c0 + CH])
        return _dot(v, p)

    def step(l, u, a, do1, do2, do3):
        b = 1 - a
        for k in range(HU):
            if do2:
                mcur = jnp.max(mb[b][k][...], axis=0, keepdims=True)
                mcur = jnp.broadcast_to(mcur, (EP, TB))
            mr = None
            for j in range(NCH):
                if do3:
                    oj = stage3(l, a, k, j)
                    if j == 0:
                        accb[k][...] = oj
                    else:
                        accb[k][...] += oj
                if do2:
                    stage2(b, k, mcur, j)
                if do1:
                    mj = stage1(l, u + 2, a, k, j)
                    mr = mj if mr is None else jnp.maximum(mr, mj)
            if do1:
                mb[a][k][...] = mr
            if do3:
                o = accb[k][...]
                o = o * (1.0 / o[DH:DH + 1, :])
                _, h = head_of(u, k)
                ot_ref[pl.ds(pl.multiple_of(h * 16, 16), 16), :] = _pack(o.astype(bf16))

    def post(t, last):
        x = xt_ref[t] + _dot(wot_ref[...], _unpack(ot_ref[...]))
        xn = _ln_t(x).astype(bf16)
        hh = jnp.maximum(_dot(w1t_ref[...], xn), 0.0).astype(bf16)
        x = x + _dot(w2t_ref[...], hh)
        if last:
            obuf_ref[t] = x.astype(bf16)
            o_copy(t).start()
        else:
            xt_ref[t] = x
            qkv(t, x, 1)

    def layer(l, c):
        def body(i, c2):
            u = i - 2
            idx = jnp.where(u < 0, i, jnp.where(u < NU - 2, 2 + (u & 1), u - (NU - 2) + 4))
            lax.switch(idx, [
                lambda: step(l, u, 0, True, False, False),
                lambda: step(l, u, 1, True, True, False),
                lambda: step(l, u, 0, True, True, True),
                lambda: step(l, u, 1, True, True, True),
                lambda: step(l, u, 0, False, True, True),
                lambda: step(l, u, 1, False, False, True),
            ])
            ispost = jnp.logical_and(u >= 0, (u & (UPT - 1)) == UPT - 1)
            t = lax.shift_right_logical(jnp.maximum(u, 0), UPT.bit_length() - 1)

            @pl.when(jnp.logical_and(ispost, l == 0))
            def _():
                post(t, False)

            @pl.when(jnp.logical_and(ispost, l == 1))
            def _():
                post(t, True)
            return c2
        lax.fori_loop(0, NU + 2, body, 0)
        return c
    lax.fori_loop(0, 2, layer, 0)
    for t in range(NT):
        o_copy(t).wait()


@jax.jit
def pallas_interleave_layers__grouped_kv_mqa__dense_activation_relu__prompt_kernel(A_x, A_wq, A_wk, A_wv, A_wo, B_x, B_w1, B_w2):
    xT = A_x.reshape(S, D).T
    scratch = [
        pltpu.VMEM((NT, D, TB), bf16),
        pltpu.VMEM((D, D), bf16),
        pltpu.VMEM((DH, D), bf16),
        pltpu.VMEM((DH, D), bf16),
        pltpu.VMEM((D, D), bf16),
        pltpu.VMEM((D, DFF), bf16),
        pltpu.VMEM((D, DFF), bf16),
        pltpu.VMEM((NT, D, TB), bf16),
        pltpu.SemaphoreType.DMA((16,)),
        pltpu.VMEM((NT, D, TB), f32),
        pltpu.VMEM((D, D), bf16),
        pltpu.VMEM((64, D), bf16),
        pltpu.VMEM((D, 512), bf16),
        pltpu.VMEM((DFF, D), bf16),
        pltpu.VMEM((512, D), f32),
        pltpu.VMEM((NT, 4, 64, TB), u32),
        pltpu.VMEM((2, 4, S // 2, 128), u32),
        pltpu.VMEM((2, NT, 16, TB), u32),
        pltpu.VMEM((256, TB), u32),
    ]
    scratch += [pltpu.VMEM((S, TB), f32)] * (2 * HU)
    scratch += [pltpu.VMEM((S // 2, TB), u32)] * (2 * HU)
    scratch += [pltpu.VMEM((8, TB), f32)] * (2 * HU)
    scratch += [pltpu.VMEM((32, TB), f32)] * HU
    outT = pl.pallas_call(
        _kernel,
        out_shape=jax.ShapeDtypeStruct((D, S), bf16),
        in_specs=[pl.BlockSpec(memory_space=pl.ANY)] * 7,
        out_specs=pl.BlockSpec(memory_space=pl.ANY),
        scratch_shapes=scratch,
        compiler_params=pltpu.CompilerParams(vmem_limit_bytes=100 * 1024 * 1024),
    )(xT, A_wq, A_wk.T, A_wv.T, A_wo, B_w1, B_w2.T)
    return outT.T.reshape(1, S, D)
```

```python
import jax
import jax.numpy as jnp
from jax import lax
import jax.experimental.pallas as pl
import jax.experimental.pallas.tpu as pltpu

f32 = jnp.float32
bf16 = jnp.bfloat16
u32 = jnp.uint32

S = 2048
D = 448
H = 16
DH = 28
DFF = 1792
TB = 512
NT = S // TB
CH = 256
NCH = S // CH
EP = 16
HU = 4
UPT = H // HU
NU = UPT * NT
QSCALE = float(DH ** -0.5 * 1.4426950408889634)
EPS = 1e-5


def _pack(x_bf16):
    return pltpu.bitcast(x_bf16, u32)


def _unpack(x_u32):
    return pltpu.bitcast(x_u32, bf16)


def _ln_t(x):
    m = jnp.mean(x, axis=0, keepdims=True)
    d = x - m
    v = jnp.mean(d * d, axis=0, keepdims=True)
    return d * lax.rsqrt(v + EPS)


def _dot(a, b):
    return jnp.dot(a, b, preferred_element_type=f32)


def _vmax(a, b):
    return b if a is None else jnp.maximum(a, b)


def _kernel(x_hbm, wq_hbm, wk_hbm, wv_hbm, wo_hbm, w1_hbm, w2_hbm, o_hbm,
            xin_ref, wq_in, wk_in, wv_in, wo_in, w1_in, w2t_ref, obuf_ref, sems,
            xt_ref, xn_ref, wqt_ref, wkv_ref, wot_ref, w1t_ref, wtmp_ref,
            qt_ref, kp_ref, vt_ref, ot_ref, *bufs):
    sb = bufs[0:HU]
    pb = bufs[HU:2 * HU]
    mb = bufs[2 * HU:3 * HU]
    accb = bufs[3 * HU:4 * HU]

    def col0(t):
        return t * TB if isinstance(t, int) else pl.multiple_of(t * TB, TB)

    def x_copy(t):
        return pltpu.make_async_copy(x_hbm.at[:, pl.ds(col0(t), TB)], xin_ref.at[t], sems.at[t])

    def o_copy(t, half):
        hb = TB // 2
        c0 = t * TB + half * hb
        c0 = c0 if isinstance(c0, int) else pl.multiple_of(c0, hb)
        return pltpu.make_async_copy(obuf_ref.at[t, :, half * hb:(half + 1) * hb],
                                     o_hbm.at[:, pl.ds(c0, hb)], sems.at[10 + 2 * t + half])

    cp_wq = pltpu.make_async_copy(wq_hbm, wq_in, sems.at[4])
    cp_wk = pltpu.make_async_copy(wk_hbm, wk_in, sems.at[5])
    cp_wv = pltpu.make_async_copy(wv_hbm, wv_in, sems.at[6])
    cp_wo = pltpu.make_async_copy(wo_hbm, wo_in, sems.at[7])
    cp_w1 = pltpu.make_async_copy(w1_hbm, w1_in, sems.at[8])
    cp_w2 = pltpu.make_async_copy(w2_hbm, w2t_ref, sems.at[9])
    cp_wk.start()
    cp_wv.start()
    cp_wq.start()
    for t in range(NT):
        x_copy(t).start()
    cp_wo.start()
    cp_w1.start()
    cp_w2.start()

    qt_ref[:, :, 56:64, :] = jnp.zeros((NT, 4, 8, TB), u32)
    wtmp_ref[...] = jnp.zeros(wtmp_ref.shape, f32)

    def ln_store(x):
        xn_ref[...] = _pack(_ln_t(x).astype(bf16))

    def qkv(t, xn, lbuf):
        rkv = _dot(wkv_ref[...], xn)
        kt = jnp.concatenate([rkv[0:32, :], jnp.zeros((96, TB), f32)], axis=0)
        k = kt.T
        row0 = pl.multiple_of(t * (TB // 2), TB // 2)
        for c in range(4):
            kc = k if c == 0 else pltpu.roll(k, c * DH, 1)
            kp_ref[lbuf, c, pl.ds(row0, TB // 2), :] = _pack(kc.astype(bf16))
        v = rkv[32:64, :]
        rows = lax.broadcasted_iota(jnp.int32, (32, TB), 0)
        v = jnp.where(rows == DH, 1.0, v)
        vt_ref[lbuf, t] = _pack(v.astype(bf16))
        rq = _dot(wqt_ref[...], xn)
        for g in range(4):
            qg = (rq[g * 112:(g + 1) * 112, :] * QSCALE).astype(bf16)
            qt_ref[t, g, 0:56, :] = _pack(qg)

    cp_wk.wait()
    cp_wv.wait()
    wtmp_ref[0:DH, :] = wk_in[...].astype(f32)
    wtmp_ref[32:32 + DH, :] = wv_in[...].astype(f32)
    wkv_ref[...] = wtmp_ref[0:64, :].astype(bf16)
    cp_wq.wait()
    wqt_ref[...] = wq_in[...].T
    x_copy(0).wait()
    x0 = xin_ref[0].astype(f32)
    xt_ref[0] = x0
    ln_store(x0)

    def pre(t, c):
        tn = jnp.minimum(t + 1, NT - 1)

        @pl.when(t + 1 < NT)
        def _():
            x_copy(tn).wait()
        xn_cur = _unpack(xn_ref[...])
        xx = xin_ref[tn].astype(f32)
        xt_ref[tn] = xx
        xn_next = _pack(_ln_t(xx).astype(bf16))
        qkv(t, xn_cur, 0)
        xn_ref[...] = xn_next
        return c
    lax.fori_loop(0, NT, pre, 0)
    cp_wo.wait()
    cp_w1.wait()
    cp_w2.wait()

    def weight_prep():
        wo32 = wo_in[...].astype(f32)
        for h in range(H):
            wtmp_ref[h * 32:h * 32 + DH, :] = wo32[h * DH:(h + 1) * DH, :]
        wot_ref[...] = wtmp_ref[...].astype(bf16).T
        w1t_ref[...] = w1_in[...].T

    def tile_of(u):
        return lax.shift_right_logical(u, UPT.bit_length() - 1)

    def stage1(l, u, k, j):
        qw = _unpack(qt_ref[tile_of(u), u & (UPT - 1)])
        kc = _unpack(kp_ref[l, k, j * (CH // 2):(j + 1) * (CH // 2), :])
        s = _dot(kc, qw)
        sb[k][j * CH:(j + 1) * CH, :] = s
        return jnp.max(s.reshape(CH // 8, 8, TB), axis=0)

    def row_max(k):
        m = jnp.max(mb[k][...], axis=0, keepdims=True)
        return jnp.broadcast_to(m, (EP, TB))

    def stage2(k, m, j):
        for r in range(j * CH, (j + 1) * CH, EP):
            p = jnp.exp2(sb[k][r:r + EP, :] - m).astype(bf16)
            pb[k][r // 2:(r + EP) // 2, :] = _pack(p)

    def stage3(l, k, j):
        p = _unpack(pb[k][j * (CH // 2):(j + 1) * (CH // 2), :])
        tt = (j * CH) // TB
        c0 = (j * CH) % TB
        v = _unpack(vt_ref[l, tt, :, c0:c0 + CH])
        oj = _dot(v, p)
        if j == 0:
            accb[k][...] = oj
        else:
            accb[k][...] += oj

    def finish(u, k):
        o = accb[k][...]
        o = o * (1.0 / o[DH:DH + 1, :])
        h = (u & (UPT - 1)) * HU + k
        ot_ref[pl.ds(pl.multiple_of(h * 16, 16), 16), :] = _pack(o.astype(bf16))

    def step(l, u, do2, do3, prep=False):
        if prep:
            weight_prep()
        for k in range(HU):
            if do2:
                mcur = row_max(k)
            mr = None
            for j in range(NCH):
                if do3:
                    stage3(l, k, j)
                if do2:
                    stage2(k, mcur, j)
                mr = _vmax(mr, stage1(l, u + 2, k, j))
            mb[k][...] = mr
            if do3:
                finish(u, k)

    def tail(l, u):
        ms = [row_max(k) for k in range(HU)]
        for k in range(HU + 1):
            for j in range(NCH):
                if k < HU:
                    stage3(l, k, j)
                    stage2(k, ms[k], j)
                if k >= 1:
                    stage3(l, k - 1, j)
            if k >= 1:
                finish(u + 1, k - 1)
            if k < HU:
                finish(u, k)

    def post(t, last):
        x = xt_ref[t] + _dot(wot_ref[...], _unpack(ot_ref[...]))
        xn = _ln_t(x).astype(bf16)
        hh = jnp.maximum(_dot(w1t_ref[...], xn), 0.0).astype(bf16)
        if last:
            hb = TB // 2
            for half in range(2):
                sl = slice(half * hb, (half + 1) * hb)
                y = x[:, sl] + _dot(w2t_ref[...], hh[:, sl])
                obuf_ref[t, :, sl] = y.astype(bf16)
                o_copy(t, half).start()
        else:
            x = x + _dot(w2t_ref[...], hh)
            xt_ref[t] = x
            qkv(t, _ln_t(x).astype(bf16), 1)

    def layer(l, c):
        def body(i, c2):
            u = i - 2
            isfull = jnp.logical_and(u >= 0, u < NU - 2)

            def other():
                lax.switch(jnp.where(u < 0, i, 2), [
                    lambda: step(l, u, False, False, prep=True),
                    lambda: step(l, u, True, False),
                    lambda: tail(l, u),
                ])
            lax.cond(isfull, lambda: step(l, u, True, True), other)
            ue = jnp.where(u == NU - 2, NU - 1, u)
            ispost = jnp.logical_and(ue >= 0, (ue & (UPT - 1)) == UPT - 1)
            t = tile_of(jnp.maximum(ue, 0))

            @pl.when(ispost)
            def _():
                lax.cond(l == 0, lambda: post(t, False), lambda: post(t, True))
            return c2
        lax.fori_loop(0, NU + 1, body, 0)
        return c
    lax.fori_loop(0, 2, layer, 0)
    for t in range(NT):
        for half in range(2):
            o_copy(t, half).wait()


@jax.jit
def pallas_interleave_layers__grouped_kv_mqa__dense_activation_relu__prompt_kernel(A_x, A_wq, A_wk, A_wv, A_wo, B_x, B_w1, B_w2):
    xT = A_x.reshape(S, D).T
    scratch = [
        pltpu.VMEM((NT, D, TB), bf16),
        pltpu.VMEM((D, D), bf16),
        pltpu.VMEM((DH, D), bf16),
        pltpu.VMEM((DH, D), bf16),
        pltpu.VMEM((D, D), bf16),
        pltpu.VMEM((D, DFF), bf16),
        pltpu.VMEM((D, DFF), bf16),
        pltpu.VMEM((NT, D, TB), bf16),
        pltpu.SemaphoreType.DMA((18,)),
        pltpu.VMEM((NT, D, TB), f32),
        pltpu.VMEM((D // 2, TB), u32),
        pltpu.VMEM((D, D), bf16),
        pltpu.VMEM((64, D), bf16),
        pltpu.VMEM((D, 512), bf16),
        pltpu.VMEM((DFF, D), bf16),
        pltpu.VMEM((512, D), f32),
        pltpu.VMEM((NT, 4, 64, TB), u32),
        pltpu.VMEM((2, 4, S // 2, 128), u32),
        pltpu.VMEM((2, NT, 16, TB), u32),
        pltpu.VMEM((256, TB), u32),
    ]
    scratch += [pltpu.VMEM((S, TB), f32)] * HU
    scratch += [pltpu.VMEM((S // 2, TB), u32)] * HU
    scratch += [pltpu.VMEM((8, TB), f32)] * HU
    scratch += [pltpu.VMEM((32, TB), f32)] * HU
    outT = pl.pallas_call(
        _kernel,
        out_shape=jax.ShapeDtypeStruct((D, S), bf16),
        in_specs=[pl.BlockSpec(memory_space=pl.ANY)] * 7,
        out_specs=pl.BlockSpec(memory_space=pl.ANY),
        scratch_shapes=scratch,
        compiler_params=pltpu.CompilerParams(vmem_limit_bytes=100 * 1024 * 1024),
    )(xT, A_wq, A_wk.T, A_wv.T, A_wo, B_w1, B_w2.T)
    return outT.T.reshape(1, S, D)
```
